```python
import os as _os
_os.environ.setdefault("JAX_PLATFORMS", "cpu")
import jax
import jax.numpy as jnp

def _softmax(x, axis=-1):
    return jax.nn.softmax(x, axis=axis)
def _gelu(x):
    return jax.nn.gelu(x, approximate=True)
def _silu(x):
    return jax.nn.silu(x)
def _sigmoid(x):
    return jax.nn.sigmoid(x)
def _layernorm(x, axis=-1, eps=1e-5):
    m = jnp.mean(x, axis=axis, keepdims=True)
    v = jnp.var(x, axis=axis, keepdims=True)
    return (x - m) / jnp.sqrt(v + eps)
def _scatter_add(tgt, idx, src, axis=0):
    return tgt.at[idx].add(src)
def _segment_sum(src, seg, n):
    return jax.ops.segment_sum(src, seg, n)
class _Rng:
    def __init__(self, key):
        self._k = key
    def _next(self):
        self._k, sub = jax.random.split(self._k)
        return sub
    def normal(self, shape):
        return jax.random.normal(self._next(), shape, dtype=jnp.bfloat16)
    def randint(self, lo, hi, shape):
        return jax.random.randint(self._next(), shape, lo, hi, dtype=jnp.int32)
    def uniform(self, shape, lo=0.0, hi=1.0):
        return jax.random.uniform(self._next(), shape, jnp.bfloat16, lo, hi)
    def permutation(self, n):
        return jax.random.permutation(self._next(), n)


kernel_name = 'interleave_layers__linear_kernel_hedgehog__sliding_block__prompt'

def setup_inputs():
    _rng = _Rng(jax.random.key(int.from_bytes(__import__("os").urandom(4), "little")))
    _w = (lambda a: (lambda t: t.astype(jnp.bfloat16) if jnp.issubdtype(t.dtype, jnp.floating) else t)(jnp.asarray(a)))
    def _A_setup():
        B, S, D, H = 1, 2048, 448, 16
        Dh = D // H
        return {
            "x": _w((lambda *s: _rng.normal(s) * 0.05)(B, S, D)),
            "wqkv": _w((lambda *s: _rng.normal(s) * 0.4)(D, 3 * D)),
            "w_phi": _w((lambda *s: _rng.normal(s) * 0.4)(H, Dh, Dh) * (Dh ** -0.5)),
            "wo": _w((lambda *s: _rng.normal(s) * 0.05)(D, D)),
        }
    _A_in = _A_setup()

    def _B_setup():
        B, S, D = 1, 2048, 448
        return {
            "x": _w((lambda *s: _rng.normal(s) * 0.05)(B, S, D)),
            "wqkv": _w((lambda *s: _rng.normal(s) * 0.1)(D, 3 * D)),
            "wo": _w((lambda *s: _rng.normal(s) * 0.1)(D, D)),
        }
    _B_in = _B_setup()

    return {
        "A_x": _A_in["x"],
        "A_wqkv": _A_in["wqkv"],
        "A_w_phi": _A_in["w_phi"],
        "A_wo": _A_in["wo"],
        "B_x": _B_in["x"],
        "B_wqkv": _B_in["wqkv"],
        "B_wo": _B_in["wo"],
    }

def reference(A_x, A_wqkv, A_w_phi, A_wo, B_x, B_wqkv, B_wo):
    def _A_ref(x, wqkv, w_phi, wo):
        B, S, D = x.shape
        H = 16; Dh = D // H
        qkv = (lambda x, *d: x.transpose(*d))((x @ wqkv).reshape(B, S, 3, H, Dh), 2, 0, 3, 1, 4)
        q, k, v = qkv[0], qkv[1], qkv[2]
        pq = jnp.einsum("bhsd,hdf->bhsf", q, w_phi)
        pk = jnp.einsum("bhsd,hdf->bhsf", k, w_phi)
        phi_q = jnp.concatenate([_softmax(pq, axis=-1), _softmax(-pq, axis=-1)], axis=-1)
        phi_k = jnp.concatenate([_softmax(pk, axis=-1), _softmax(-pk, axis=-1)], axis=-1)
        kv = jnp.einsum("bhsf,bhsd->bhfd", phi_k, v)
        z  = jnp.einsum("bhsf->bhf", phi_k)
        num = jnp.einsum("bhqf,bhfd->bhqd", phi_q, kv)
        den = jnp.einsum("bhqf,bhf->bhq", phi_q, z)[..., None] + 1e-6
        o = num / den
        return (lambda x, *d: x.transpose(*d))(o, 0, 2, 1, 3).reshape(B, S, D) @ wo

    def _B_ref(x, wqkv, wo):
        B, S, D = x.shape
        H = 16; Dh = D // H; W = 256
        qkv = (lambda x, *d: x.transpose(*d))((x @ wqkv).reshape(B, S, 3, H, Dh), 2, 0, 3, 1, 4)
        q, k, v = qkv[0], qkv[1], qkv[2]
        scores = jnp.einsum("bhqd,bhkd->bhqk", q, k) * (Dh ** -0.5)
        idx = jnp.arange(S)
        mask = (idx[:, None] - idx[None, :] >= 0) & (idx[:, None] - idx[None, :] < W)
        scores = jnp.where(mask[None, None], scores, -1e9)
        p = _softmax(scores, axis=-1)
        o = jnp.einsum("bhqk,bhkd->bhqd", p, v)
        return (lambda x, *d: x.transpose(*d))(o, 0, 2, 1, 3).reshape(B, S, D) @ wo

    x = A_x
    x = x + _A_ref(_layernorm(x, axis=-1), A_wqkv, A_w_phi, A_wo)
    x = x + _B_ref(_layernorm(x, axis=-1), B_wqkv, B_wo)
    x = x + _A_ref(_layernorm(x, axis=-1), A_wqkv, A_w_phi, A_wo)
    x = x + _B_ref(_layernorm(x, axis=-1), B_wqkv, B_wo)
    return x
```

```python
import functools
import itertools
import math

import jax
import jax.numpy as jnp
from jax import lax
import jax.experimental.pallas as pl
import jax.experimental.pallas.tpu as pltpu

F32, BF16, I32 = jnp.float32, jnp.bfloat16, jnp.int32
H, DH, WIN = 16, 28, 256
D = H * DH
PAIR, GRP = 2 * DH, 4 * DH
LANES = 128
QB = 32
LOG2E = math.log2(math.e)
NEG = -1e30
T = 512
PART = (WIN + QB) // 3

LAG_A, RATE_A = 16, 0.49
LAG_NA, LAG_NB = 0, 28
LAG_EXP = (10, 11, 10)
SLOT_B, SLOT_O = 2, 3
HEAD_A = 6
AHEAD = 7
FILL_O = (48, 49, 51, 52, 54)
OUTER_O = (2, 4, 1, 5, 7, 3, 6)
OUTER_A = OUTER_B = ONCE = (2, 4, 5, 1, 7, 3, 6)
WAITS = ((0, 1), (2, 3))
UNITS = [(g, i) for half in ((0, 1), (2, 3)) for gs in ((2, 3), (0, 1)) for i in half for g in gs]
NT_DIMS = (((1,), (1,)), ((), ()))


def _iota(shape, dim):
    return lax.broadcasted_iota(I32, shape, dim)


def _mm(a, b):
    return jnp.dot(a, b, preferred_element_type=F32)


def _mm_nt(a, b):
    return lax.dot_general(a, b, NT_DIMS, preferred_element_type=F32)


def _tiles(x):
    return [x[r:r + 8] for r in range(0, x.shape[0], 8)]


def _tree(op, xs):
    while len(xs) > 1:
        xs = [op(*xs[i:i + 2]) if i + 1 < len(xs) else xs[i] for i in range(0, len(xs), 2)]
    return xs[0]


def _all_sublanes(op, v, shifts):
    for s in shifts:
        v = op(v, pltpu.roll(v, s, 0))
    return v


def _recip(x):
    return pl.reciprocal(x, approx=True)


def _moments(x, gate=lambda t: t):
    rows = _tiles(x)
    mean = gate(_tree(jnp.add, rows)) * (1.0 / len(rows))
    return mean, _tree(jnp.add, [(r - mean) * (r - mean) for r in rows])


def _norm_stats(moments):
    means, squares = zip(*moments)
    mean = _all_sublanes(jnp.add, _tree(jnp.add, means), (4, 2, 1)) * (1.0 / 32)
    between = _tree(jnp.add, [(m - mean) * (m - mean) for m in means]) * (D / 32)
    var = _all_sublanes(jnp.add, _tree(jnp.add, squares) + between, (4, 2, 1)) * (1.0 / D)
    return mean, lax.rsqrt(var + 1e-5)


def _hedgehog(p, gate, scaled=False):
    rows = _tiles(p)
    first = gate(rows[0])
    hi = _all_sublanes(jnp.maximum, functools.reduce(jnp.maximum, rows[1:], first), (4, 2))
    lo = _all_sublanes(jnp.minimum, functools.reduce(jnp.minimum, rows[1:], first), (4, 2))
    pos, neg = [jnp.exp2(r - hi) for r in rows], [jnp.exp2(lo - r) for r in rows]
    pos_sum, neg_sum = (_all_sublanes(jnp.add, _tree(jnp.add, e), (4, 2)) for e in (pos, neg))
    if scaled:
        ratio = pos_sum * _recip(neg_sum)
        out = pos + [v * ratio for v in neg] + [pos_sum, pos_sum]
    else:
        pos_inv, neg_inv = _recip(pos_sum), _recip(neg_sum)
        out = [v * pos_inv for v in pos] + [v * neg_inv for v in neg]
    return jnp.concatenate(out, 0).astype(BF16)


_LEFT = {1: ((0, 1), (3, 1)), 2: ((2, 1), (3, 1)), 3: ((0, 1),), 4: ((3, 1),),
         5: ((0, 1), (1, 1)), 6: ((2, 1), (0, -1)), 7: ((1, 1), (3, -1))}
_RIGHT = {1: ((0, 1), (3, 1)), 2: ((0, 1),), 3: ((1, 1), (3, -1)), 4: ((2, 1), (0, -1)),
          5: ((3, 1),), 6: ((0, 1), (1, 1)), 7: ((2, 1), (3, 1))}
_RESULT = ({1: 1, 4: 1, 5: -1, 7: 1}, {3: 1, 5: 1}, {2: 1, 4: 1}, {1: 1, 2: -1, 3: 1, 6: 1})
_INNER = (((2, 4, 5, 3), (1, 7, 6)), ((1, 7, 6), (2, 4, 5, 3)),
          ((3, 6), (1, 2, 4, 5), (7,)), ((7,), (1, 4, 5, 2), (3, 6)))


def _signed_sum(terms):
    (out, sign), *rest = terms
    for value, s in rest:
        if s == sign:
            out = out + value
        elif sign > 0:
            out = out - value
        else:
            out, sign = value - out, 1
    return out, sign


def _factors(terms, block):
    @functools.cache
    def quadrant(outer, q):
        return _signed_sum([(block(2 * (o // 2) + q // 2, 2 * (o % 2) + q % 2, outer), s)
                            for o, s in terms[outer]])[0]

    return lambda outer, inner: _signed_sum([(quadrant(outer, q), s) for q, s in terms[inner]])[0]


def _right_factors(block):
    pad = jnp.zeros((LANES - GRP, LANES), F32)
    factor = _factors(_RIGHT, block)
    return functools.cache(lambda *k: jnp.concatenate([factor(*k), pad], 0).astype(BF16))


def _factor_lanes(outer, inner):
    return pl.ds((7 * outer + inner - 8) * LANES, LANES)


def _strassen(left, right, done, clock, slot, sequence):
    products = [{} for _ in range(4)]
    for outer in sequence:
        partial, seen = [[] for _ in range(4)], set()
        for together in _INNER[slot % 4]:
            m = {}
            for inner in together:
                m[inner] = _mm(left(_factor_lanes(outer, inner)), right(outer, inner))
                if slot % 4 == 0:
                    clock.extend(m[inner][r:r + 8] for r in range(0, m[inner].shape[0] - 16, 32))
                slot += 1
                if inner != together[-1]:
                    yield
            seen.update(together)
            for q, result in enumerate(_RESULT):
                new = [(m[k], s) for k, s in result.items() if k in m]
                if not new:
                    continue
                partial[q] = [_signed_sum(new + partial[q])]
                if seen.issuperset(result):
                    products[q][outer] = partial[q][0][0]
                    for o, total in enumerate(_RESULT):
                        if outer in total and all(k in products[q] for k in total):
                            order = [outer] + [k for k in total if k != outer]
                            done(2 * (o // 2) + q // 2, 2 * (o % 2) + q % 2,
                                 _signed_sum([(products[q][k], total[k]) for k in order])[0])
            yield


def _strassen_once(left, block, done, clock):
    pad = jnp.zeros((LANES - GRP, LANES), F32)
    for half in range(2):
        m = {}
        for inner in ONCE:
            right = [_signed_sum([(block(2 * k + q // 2, 2 * half + q % 2), s) for q, s in _RIGHT[inner]])[0]
                     for k in range(2)]
            right = jnp.concatenate([right[0], pad, right[1], pad], 0).astype(BF16)
            m[inner] = _mm(left(pl.ds((inner - 1) * 2 * LANES, 2 * LANES)), right)
            clock.extend(m[inner][r:r + 8] for r in range(0, 2 * GRP, 64))
            for q, total in enumerate(_RESULT):
                if inner in total and all(k in m for k in total):
                    order = [k for k in ONCE[::-1] if k in total]
                    y = _signed_sum([(m[k], total[k]) for k in order])[0]
                    for r in range(2):
                        done(2 * r + q // 2, 2 * half + q % 2, y[r * GRP:(r + 1) * GRP])
            yield


def _schedule(ahead):
    order = "nnn" + "a" * HEAD_A + "n" + "a" * (14 - HEAD_A) + "b" * 49
    for n in range(48 + ahead):
        order += "s" * (n < 48) + "oooo" * (n in FILL_O) + "p" * (n >= ahead)
    return order + "o" * (49 - 4 * len(FILL_O))


def _pack(x):
    return pltpu.bitcast(x.astype(BF16), I32)


def _unpack(x):
    return pltpu.bitcast(x, BF16)


def _head_in_group(i):
    return (i >= DH).astype(I32) + (i >= 2 * DH).astype(I32) + (i >= 3 * DH).astype(I32)


def _kernel(x_hbm, wa_hbm, wphi_hbm, woa_hbm, wb_hbm, wob_hbm, out_hbm,
            xio, wa_raw, wphi_raw, woa_raw, wb_raw, wob_raw,
            plain, mapped, wa, woa, wb, wob, xres, phiq, kv_acc, kv_mat, kbuf, vbuf, pbuf, qbuf, qmask,
            sem_x, sem_w, sem_o, *, nch):
    nb = T // LANES
    wa, woa, wb, wob, phiq, vbuf, pbuf = (
        w.bitcast(BF16) for w in (wa, woa, wb, wob, phiq, vbuf, pbuf))

    def aligned(start, size):
        return pl.ds(start if isinstance(start, int) else pl.multiple_of(start, size), size)

    def x_copy(c):
        return pltpu.make_async_copy(x_hbm.at[:, aligned(c * T, T)], xio.at[c], sem_x.at[c])

    def load_x(c):
        x_copy(c).wait()
        for i in range(nb):
            xres[c * nb + i] = xio[c, :, pl.ds(i * LANES, LANES)].astype(F32)

    def out_copy(c, quad):
        rows, lanes = pl.ds(quad // 2 * (D // 2), D // 2), quad % 2 * (T // 2)
        return pltpu.make_async_copy(xio.at[c, rows, pl.ds(lanes, T // 2)],
                                     out_hbm.at[rows, aligned(c * T + lanes, T // 2)], sem_o.at[4 * c + quad])

    def wait_output():
        for c in range(nch):
            for quad in range(4):
                out_copy(c, quad).wait()

    def rest_copies(k):
        rows = aligned(k * GRP, GRP)
        return [pltpu.make_async_copy(src.at[rows, :], dst.at[rows, :], sem_w.at[1 + 3 * k + n])
                for n, (src, dst) in enumerate(((woa_hbm, woa_raw), (wob_hbm, wob_raw), (wb_hbm, wb_raw)))]

    phi_copy = pltpu.make_async_copy(wphi_hbm, wphi_raw, sem_w.at[0])
    wa_copies = [pltpu.make_async_copy(wa_hbm.at[aligned(k * GRP, GRP), :], wa_raw.at[aligned(k * GRP, GRP), :],
                                       sem_w.at[13 + k]) for k in range(4)]
    phi_copy.start()
    for cp in wa_copies:
        cp.start()

    row, lane = 2 * _iota((LANES // 2, LANES), 0), _iota((LANES // 2, LANES), 1)
    for c in range(4):
        keep = ((_head_in_group(row) + c) & 3) == (lane >> 5)
        qmask[c] = jnp.where(keep, -1, 0)

    phi_copy.wait()
    r, c_ = _iota((D, D), 0), _iota((D, D), 1)
    perm = jnp.where((c_ & (H - 1)) * DH + (c_ >> 4) == r, 1.0, 0.0).astype(BF16)
    wphi = _mm(perm, wphi_raw[...]).astype(BF16)
    r, c_ = _iota((GRP, DH), 0), _iota((GRP, DH), 1)
    spread = jnp.where((jnp.where(r >= PAIR, r - PAIR, r) >> 1) == c_, 1.0, 0.0).astype(BF16)
    r, c_ = _iota((GRP, GRP), 0), _iota((GRP, GRP), 1)
    same_head = jnp.where(r >= PAIR, 2, 0) + (r & 1) == _head_in_group(c_)
    fold = [jnp.where(same_head, _mm_nt(spread, wphi[g * GRP:(g + 1) * GRP]), 0.0).astype(BF16)
            for g in range(4)]

    def transpose(raw, k, start, folded=0):
        pad = jnp.zeros((LANES - GRP, raw.shape[1]), BF16)
        cols = jnp.concatenate([raw[aligned(k * GRP, GRP), :], pad], 0).T
        for n in range(4 * folded):
            mapped[k, n * GRP:(n + 1) * GRP, :] = _mm(fold[n % 4], cols[n * GRP:(n + 1) * GRP]) * LOG2E
        plain[k, pl.ds(start, raw.shape[1] - folded * D), :] = cols[folded * D:]

    def left_factors(src, start, dst, part):
        def body(r, carry):
            r = pl.multiple_of(r * 16, 16)

            @functools.cache
            def block(g, k):
                w = src[k, pl.ds(start + g * GRP + r, 16), :].astype(F32)
                return w * (DH ** -0.5 * LOG2E) if dst is wb and part == 0 else w

            if dst is woa:
                for inner, g, k in itertools.product(_LEFT, range(2), range(2)):
                    f = _signed_sum([(block(2 * g + q // 2, 2 * k + q % 2), s) for q, s in _LEFT[inner]])[0]
                    dst[pl.ds(g * GRP + r, 16), pl.ds((2 * inner - 2 + k) * LANES, LANES)] = f.astype(BF16)
                return carry
            factor = _factors(_LEFT, lambda g, k, _: block(g, k))
            for outer in _LEFT:
                for inner in _LEFT:
                    dst[pl.ds(part * GRP + r, 16), _factor_lanes(outer, inner)] = factor(outer, inner).astype(BF16)
            return carry

        lax.fori_loop(0, GRP // 16, body, 0)

    for n, ks in enumerate(WAITS):
        for k in ks:
            wa_copies[k].wait()
        if n == 0:
            for cp in [x_copy(0), x_copy(1)] + rest_copies(0):
                cp.start()
        for k in ks:
            transpose(wa_raw, k, 0, 2)
    left_factors(mapped, 0, wa, 0)
    left_factors(mapped, D, wa, 1)
    left_factors(plain, 0, wa, 2)

    def prepare_rest():
        for n, (dst, part) in enumerate(((woa, 0), (wob, 0), (wb, 0), (wb, 1), (wb, 2))):
            left_factors(plain, n * D, dst, part)

    low = _iota((8, LANES), 0) < 4

    clock = []

    def after(x, lag):
        if not lag or len(clock) < lag:
            return x
        return tied(x, clock[-lag])

    def tied(x, other):
        return jnp.where(qmask[0, 0:8, :] > 0, other, x)

    def normalized(block, stats, lag):
        @functools.cache
        def get(k, i, outer):
            mean, inv = stats(i)
            inv = after(inv, lag)
            shift = mean * inv
            return jnp.concatenate([r * inv - shift for r in _tiles(block(k, i))], 0)

        return _right_factors(lambda k, i, outer: get(k, i, outer if lag else 0))

    def gate(t):
        return after(t, LAG_A)

    def paced(steps, jobs, rate):
        credit = 0.0
        for _ in steps:
            credit = min(credit + rate, 2.0)
            while jobs and credit >= 1:
                jobs.pop(0)()
                credit -= 1
            yield

    def a_features(layer, c, stats):
        @pl.when(layer == 0)
        def _():
            pl.when(c + 1 < nch)(lambda: load_x(c + 1))
            for cp in rest_copies(c):
                cp.wait()

        ones = jnp.ones((8, LANES), F32)
        phik, values, moments = {}, {}, []
        clock.clear()

        def features(part, p, i, x):
            if part == 0:
                phiq[c * nb + i, :, pl.ds(p * LANES, LANES)] = _hedgehog(x, gate, True)
            else:
                phik[p, i] = _hedgehog(x, gate)

        def next_moments(i, gs):
            blk = jnp.minimum(c + 1, nch - 1) * nb + i
            moments.extend(_moments(xres[blk, pl.ds(g * GRP, GRP), :], gate) for g in gs)

        def done(part, g, i, y):
            for j in range(2):
                x = y[j * PAIR:(j + 1) * PAIR]
                if part < 2:
                    jobs.append(functools.partial(features, part, 2 * g + j, i, x))
                else:
                    values[2 * g + j, i] = jnp.concatenate([x, ones], 0).astype(BF16)

        right = normalized(lambda k, i: xres[c * nb + i, pl.ds(k * GRP, GRP), :], stats.__getitem__, LAG_NA)
        jobs = [functools.partial(next_moments, i, gs) for i in range(nb) for gs in ((0, 1), (2, 3))]
        total = {}

        def steps():
            for n, part in enumerate((1, 0, 2)):
                left = lambda lanes, part=part: wa[pl.ds(part * GRP, GRP), lanes]
                yield from _strassen(left, right, functools.partial(done, part), clock, n, OUTER_A)
            for n, (p, i) in enumerate(values):
                part = _mm_nt(values[p, i], phik[p, i])
                total[p] = (total[p] if p in total else kv_acc[p]) + part
                if n % 2:
                    clock.append(jnp.concatenate([part[:8], part[:8, :LANES - GRP]], 1))
                    yield

        for _ in paced(steps(), jobs, RATE_A):
            pass
        for job in jobs:
            job()
        for raw, start in ((woa_raw, 0), (wob_raw, D), (wb_raw, 2 * D)):
            transpose(raw, c, start)
        for p in range(H // 2):
            kv_acc[p] = total[p]
        return [_norm_stats(moments[4 * i:4 * i + 4]) for i in range(nb)]

    def a_finish_kv():
        r, c_ = _iota((64, LANES), 0), _iota((64, LANES), 1)
        second = ((r >= DH) & (r < PAIR)) | (r >= PAIR + 4)
        keep = second.astype(I32) == (c_ & 1)
        eps = jnp.where((r >= PAIR) & (c_ < 2), 1e-6, 0.0)[:, :LANES - GRP]
        for p in range(H // 2):
            kv_mat[p] = _pack(jnp.where(keep, jnp.concatenate([kv_acc[p], eps], 1), 0.0))

    def rot(t, h):
        return pltpu.roll(t, QB * h, 1) if h else t

    def a_heads(st, c):
        for i in range(nb):
            for g in range(4):
                o = []
                for p in (2 * g, 2 * g + 1):
                    phi = phiq[c * nb + i, :, pl.ds(p * LANES, LANES)]
                    nd = _tiles(_mm(_unpack(kv_mat[p]), phi))
                    inv = _recip(nd[7])
                    swapped = pltpu.roll(inv, 4, 0)
                    inv_a, inv_b = jnp.where(low, inv, swapped), jnp.where(low, swapped, inv)
                    o += [t * inv_a for t in nd[0:3]] + [nd[3] * inv] + [t * inv_b for t in nd[4:7]]
                st["oa", g, i] = jnp.concatenate(o, 0)
            yield

    def a_output(st, c):
        def done(g, i, y):
            st["x", g, i] = xres[c * nb + i, pl.ds(g * GRP, GRP), :] + y
            st["moments", g, i] = _moments(st["x", g, i])
            if all(("x", k, i) in st for k in range(4)):
                st["stats", i] = _norm_stats([st["moments", k, i] for k in range(4)])

        return _strassen_once(lambda n: woa[:, n], lambda k, i: st["oa", k, i], done, clock)

    def b_project(st, c):
        def done(g, i, qkv):
            q = _tiles(qkv[:GRP])
            qr = []
            for j in range(2):
                t = q[7 * j:7 * j + 7]
                qr += [rot(u, 2 * j) for u in t[0:3]]
                qr.append(jnp.where(low, rot(t[3], 2 * j), rot(t[3], 2 * j + 1)))
                qr += [rot(u, 2 * j + 1) for u in t[4:7]]
            qr.append(jnp.zeros((LANES - GRP, LANES), F32))
            qr = _pack(jnp.concatenate(qr, 0))
            for m in range(4):
                qbuf[4 * i + g, m] = qr & qmask[m]
            k = jnp.concatenate([qkv[GRP:2 * GRP], jnp.zeros((LANES - GRP, LANES), F32)], 0)
            kbuf[g, pl.ds((WIN + i * LANES) // 2, LANES // 2), :] = _pack(k.astype(BF16).T)
            v = _tiles(qkv[2 * GRP:])
            ve = []
            for t in (v[:7], v[7:]):
                ve += t[0:3] + [jnp.where(low, t[3], 1.0), jnp.where(low, 1.0, t[3])] + t[4:7]
            vbuf[pl.ds(g * LANES, LANES), pl.ds(WIN + i * LANES, LANES)] = (
                jnp.concatenate(ve, 0).astype(BF16))

        right = normalized(lambda k, i: st["x", k, i], lambda i: st["stats", i], LAG_NB)
        return _strassen(lambda n: wb[:, n], right, done, clock, SLOT_B, OUTER_B)

    newer = [_iota((8, LANES), 0) + r <= (_iota((8, LANES), 1) & (QB - 1)) for r in range(0, QB, 8)]
    lane_grp = _iota((8, LANES), 1) >> 5

    def b_scores(st, begin):
        for g, i in UNITS:
            s = [{} for _ in range(4)]
            top = [None] * 4
            for part in range(3):
                raw = []
                for m in range(4):
                    oldest = i * LANES + m * QB
                    lo, hi = max(oldest + part * PART, begin), oldest + (part + 1) * PART
                    if hi <= lo:
                        continue
                    raw = _tiles(_mm(_unpack(kbuf[g, lo // 2:hi // 2, :]), _unpack(qbuf[4 * i + g, m])))
                    for n, t in enumerate(raw, (lo - oldest) // 8):
                        if n >= WIN // 8:
                            t = jnp.where(newer[n - WIN // 8], t, s[m].get(n - WIN // 8, NEG))
                        if n >= QB // 8:
                            top[m] = t if top[m] is None else jnp.maximum(top[m], t)
                        s[m][n] = t
                clock.extend(raw[::4])
                if part == 2:
                    st["s", g, i] = s, [_all_sublanes(jnp.maximum, t, (4, 2, 1)) for t in top]
                yield

    def pick(mask, a, b):
        if a is None and b is None:
            return None
        return jnp.where(mask, 0 if a is None else a, 0 if b is None else b)

    def packed(x, row, col):
        at = pl.ds(16 * row, 16), pl.ds(col * LANES, LANES)
        pbuf[at] = x.astype(BF16)
        return pltpu.bitcast(pbuf[at], I32)

    def b_heads(st, begin):
        for g, i in UNITS:
            o = []
            s, top = st["s", g, i]
            edge = {}
            acc = [None] * 4

            def weight(m, n):
                r = n - m * (QB // 8)
                if QB // 8 <= r < WIN // 8:
                    return jnp.exp2(s[m][r] - top[m])
                k = r % (WIN // 8)
                if (m, k) not in edge:
                    edge[m, k] = jnp.exp2(s[m][WIN // 8 + k] - top[m])
                return jnp.where(newer[k], 0.0, edge[m, k]) if r == k else jnp.where(newer[k], edge[m, k], 0.0)

            for j in range(3):
                if (i + j) * LANES < begin:
                    yield
                    continue
                top = [after(t, LAG_EXP[j]) for t in top]
                probs = [[] for _ in range(4)]
                for n in range(16 * j, 16 * j + 16, 2):
                    e = [packed(jnp.concatenate([weight(m, n), weight(m, n + 1)], 0), n // 2, m)
                         if 0 <= 8 * n - m * QB < WIN + QB else None for m in range(4)]
                    for h0 in range(2):
                        even = (lane_grp & 1) == h0
                        u = [pick(even, e[0], e[1]), pick(even, e[2], e[3])]
                        for h in (h0, h0 + 2):
                            probs[h].append(pick(((lane_grp - h) & 2) == 0, u[0], u[1]))
                for h in range(4):
                    vt = vbuf[pl.ds((4 * g + h) * 32, 32), pl.ds((i + j) * LANES, LANES)]
                    part = _mm(vt, _unpack(jnp.concatenate(probs[h], 0)))
                    acc[h] = part if acc[h] is None else acc[h] + part
                clock.append(part[:8])
                if j < 2:
                    yield
            for h in range(4):
                t = _tiles(acc[h])
                den = t[3] if h % 2 == 0 else t[0]
                swapped = pltpu.roll(den, 4, 0)
                inv = _recip(jnp.where(low, swapped, den) if h % 2 == 0 else jnp.where(low, den, swapped))
                t = [rot(u * inv, (4 - h) % 4) for u in t]
                if h % 2 == 0:
                    o += t
                else:
                    o += [jnp.where(low, o.pop(), t[0])] + t[1:]
            st["ob", g, i] = jnp.concatenate(o, 0)
            yield

    def b_output(st, c):
        written = []

        def done(g, i, y):
            y = st["x", g, i] + y
            xres[c * nb + i, pl.ds(g * GRP, GRP), :] = y
            xio[c, pl.ds(g * GRP, GRP), pl.ds(i * LANES, LANES)] = y.astype(BF16)
            written.append(g // 2 * 2 + i // 2)
            if written.count(written[-1]) == 4:
                out_copy(c, written[-1]).start()

        return _strassen(lambda n: wob[:, n], _right_factors(lambda k, i, _: st["ob", k, i]), done, clock, SLOT_O, OUTER_O)

    def second_half(c, layer):
        begin = WIN if isinstance(c, int) else 0
        if not begin:
            for g in range(4):
                kbuf[g, 0:WIN // 2, :] = kbuf[g, T // 2:(T + WIN) // 2, :]
            vbuf[:, 0:WIN] = vbuf[:, T:T + WIN]
        st = {}
        clock.clear()
        running = dict(n=a_heads(st, c), a=a_output(st, c), b=b_project(st, c), s=b_scores(st, begin),
                       p=b_heads(st, begin), o=b_output(st, c))
        for step in _schedule(AHEAD):
            next(running[step])
        assert all(next(stage, True) for stage in running.values())
        return layer

    load_x(0)
    for c in range(1, nch):
        for cp in rest_copies(c) + ([x_copy(c + 1)] if c + 1 < nch else []):
            cp.start()

    def layer_pair(layer, carry):
        kv_acc[...] = jnp.zeros(kv_acc.shape, F32)
        moments = [_moments(xres[i, pl.ds(g * GRP, GRP), :]) for i in range(nb) for g in range(4)]
        lax.fori_loop(0, nch, functools.partial(a_features, layer), [_norm_stats(moments[4 * i:4 * i + 4]) for i in range(nb)])
        pl.when(layer == 0)(prepare_rest)
        pl.when(layer == 1)(wait_output)
        a_finish_kv()
        lax.fori_loop(1, nch, second_half, second_half(0, layer))
        return carry

    lax.fori_loop(0, 2, layer_pair, 0)
    wait_output()


@jax.jit
def pallas_interleave_layers__linear_kernel_hedgehog__sliding_block__prompt_kernel(
    A_x: jax.Array,
    A_wqkv: jax.Array,
    A_w_phi: jax.Array,
    A_wo: jax.Array,
    B_x: jax.Array,
    B_wqkv: jax.Array,
    B_wo: jax.Array,
):
    del B_x
    _, seq, _ = A_x.shape
    nch = seq // T
    assert nch == 4
    vmem = pltpu.VMEM
    out = pl.pallas_call(
        functools.partial(_kernel, nch=nch),
        in_specs=[pl.BlockSpec(memory_space=pl.ANY)] * 6,
        out_specs=pl.BlockSpec(memory_space=pl.ANY),
        out_shape=jax.ShapeDtypeStruct((D, seq), BF16),
        scratch_shapes=[
            vmem((nch, D, T), BF16),
            vmem((D, 3 * D), BF16), vmem((D, DH), BF16), vmem((D, D), BF16),
            vmem((D, 3 * D), BF16), vmem((D, D), BF16),
            vmem((4, 5 * D, LANES), BF16), vmem((4, 2 * D, LANES), F32),
            vmem((3 * PAIR, 49 * LANES), I32), vmem((GRP, 14 * LANES), I32),
            vmem((3 * PAIR, 49 * LANES), I32), vmem((PAIR, 49 * LANES), I32),
            vmem((seq // LANES, D, LANES), F32),
            vmem((seq // LANES, LANES // 2, H // 2 * LANES), I32),
            vmem((H // 2, 64, GRP), F32), vmem((H // 2, 32, LANES), I32),
            vmem((4, (WIN + T) // 2, LANES), I32),
            vmem((H * 16, WIN + T), I32), vmem((3 * LANES // 2, 4 * LANES), I32),
            vmem((4 * T // LANES, 4, LANES // 2, LANES), I32), vmem((4, LANES // 2, LANES), I32),
            pltpu.SemaphoreType.DMA((nch,)), pltpu.SemaphoreType.DMA((17,)),
            pltpu.SemaphoreType.DMA((4 * nch,)),
        ],
        compiler_params=pltpu.CompilerParams(vmem_limit_bytes=100 * 1024 * 1024),
    )(A_x[0].T, A_wqkv, A_w_phi.transpose(1, 0, 2).reshape(D, DH), A_wo, B_wqkv, B_wo)
    return out.T[None].astype(A_x.dtype)
```
